```python
import os as _os
_os.environ.setdefault("JAX_PLATFORMS", "cpu")
import jax
import jax.numpy as jnp

def _softmax(x, axis=-1):
    return jax.nn.softmax(x, axis=axis)
def _gelu(x):
    return jax.nn.gelu(x, approximate=True)
def _silu(x):
    return jax.nn.silu(x)
def _sigmoid(x):
    return jax.nn.sigmoid(x)
def _layernorm(x, axis=-1, eps=1e-5):
    m = jnp.mean(x, axis=axis, keepdims=True)
    v = jnp.var(x, axis=axis, keepdims=True)
    return (x - m) / jnp.sqrt(v + eps)
def _scatter_add(tgt, idx, src, axis=0):
    return tgt.at[idx].add(src)
def _segment_sum(src, seg, n):
    return jax.ops.segment_sum(src, seg, n)
class _Rng:
    def __init__(self, key):
        self._k = key
    def _next(self):
        self._k, sub = jax.random.split(self._k)
        return sub
    def normal(self, shape):
        return jax.random.normal(self._next(), shape, dtype=jnp.bfloat16)
    def randint(self, lo, hi, shape):
        return jax.random.randint(self._next(), shape, lo, hi, dtype=jnp.int32)
    def uniform(self, shape, lo=0.0, hi=1.0):
        return jax.random.uniform(self._next(), shape, jnp.bfloat16, lo, hi)
    def permutation(self, n):
        return jax.random.permutation(self._next(), n)


kernel_name = 'gated_mix__compressed_kv_cla__linear_attn_block__prompt'

def setup_inputs():
    _rng = _Rng(jax.random.key(int.from_bytes(__import__("os").urandom(4), "little")))
    _w = (lambda a: (lambda t: t.astype(jnp.bfloat16) if jnp.issubdtype(t.dtype, jnp.floating) else t)(jnp.asarray(a)))
    def _A_setup():
        B, H, Sq, Sk, D, M = 1, 16, 2048, 2048, 256, 448
        Dc = 4 * D
        return {
            "x": _w((lambda *s: _rng.normal(s) * 0.05)(B, Sq, M)),
            "c_kv": _w((lambda *s: _rng.normal(s) * 0.8)(B, Sk, Dc)),
            "w_q": _w((lambda *s: _rng.normal(s) * 3.2)(M, H, D) * (M ** -0.5)),
            "w_uk": _w((lambda *s: _rng.normal(s) * 3.2)(Dc, H, D) * (Dc ** -0.5)),
            "w_uv": _w((lambda *s: _rng.normal(s) * 0.8)(Dc, H, D) * (Dc ** -0.5)),
            "w_o": _w((lambda *s: _rng.normal(s) * 0.8)(H, D, M) * ((H * D) ** -0.5)),
        }
    _A_in = _A_setup()

    def _B_setup():
        B, S, D = 1, 2048, 448
        return {
            "x": _w((lambda *s: _rng.normal(s) * 0.05)(B, S, D)),
            "wqkv": _w((lambda *s: _rng.normal(s) * 1.6)(D, 3 * D)),
            "wo": _w((lambda *s: _rng.normal(s) * 0.4)(D, D)),
        }
    _B_in = _B_setup()

    return {
        "A_x": _A_in["x"],
        "A_c_kv": _A_in["c_kv"],
        "A_w_q": _A_in["w_q"],
        "A_w_uk": _A_in["w_uk"],
        "A_w_uv": _A_in["w_uv"],
        "A_w_o": _A_in["w_o"],
        "B_x": _B_in["x"],
        "B_wqkv": _B_in["wqkv"],
        "B_wo": _B_in["wo"],
        "gate_w": _w((lambda *s: _rng.normal(s) * 0.05)(448) * 16.0),
    }

def reference(A_x, A_c_kv, A_w_q, A_w_uk, A_w_uv, A_w_o, B_x, B_wqkv, B_wo, gate_w):
    def _A_ref(x, c_kv, w_q, w_uk, w_uv, w_o):
        B, Sq, M = x.shape[0], x.shape[1], x.shape[2]
        Sk = c_kv.shape[1]
        H, D = w_q.shape[1], w_q.shape[2]
        q = jnp.einsum("bqm,mhd->bhqd", x, w_q)
        k = jnp.einsum("bkc,chd->bhkd", c_kv, w_uk)
        v = jnp.einsum("bkc,chd->bhkd", c_kv, w_uv)
        scores = jnp.einsum("bhqd,bhkd->bhqk", q, k) * (D ** -0.5)
        off = Sk - Sq
        qi = jnp.arange(Sq)[:, None]
        kj = jnp.arange(Sk)[None, :]
        cmask = kj <= (qi + off)
        scores = jnp.where(cmask[None, None], scores, -1e9)
        p = _softmax(scores, axis=-1)
        ctx = jnp.einsum("bhqk,bhkd->bhqd", p, v)
        return jnp.einsum("bhqd,hdm->bqm", ctx, w_o)

    def _B_ref(x, wqkv, wo):
        B, S, D = x.shape
        H = 16; Dh = D // H
        qkv = (lambda x, *d: x.transpose(*d))((x @ wqkv).reshape(B, S, 3, H, Dh), 2, 0, 3, 1, 4)
        q, k, v = qkv[0], qkv[1], qkv[2]
        phi = lambda t: jnp.where(t > 0, t + 1, jnp.exp(t)) + 1e-6
        pq, pk = phi(q), phi(k)
        kv = jnp.einsum("bhsd,bhse->bhde", pk, v)
        z = jnp.einsum("bhsd->bhd", pk)
        num = jnp.einsum("bhqd,bhde->bhqe", pq, kv)
        den = jnp.einsum("bhqd,bhd->bhq", pq, z)[..., None] + 1e-6
        o = num / den
        return (lambda x, *d: x.transpose(*d))(o, 0, 2, 1, 3).reshape(B, S, D) @ wo

    x = A_x
    g = _sigmoid((x * gate_w).sum(-1, keepdims=True))
    a = _A_ref(x, A_c_kv, A_w_q, A_w_uk, A_w_uv, A_w_o)
    b = _B_ref(x, B_wqkv, B_wo)
    return g * a + (1 - g) * b
```

```python
import functools
import jax
import jax.numpy as jnp
from jax import lax
import jax.experimental.pallas as pl
import jax.experimental.pallas.tpu as pltpu

S = 2048
M = 448
H = 16
D = 256
C = 1024
DH = 28
NT = S // 128
NEG = -1e30
LOG2E = 1.4426950408889634
f32, bf16, i32 = jnp.float32, jnp.bfloat16, jnp.int32


def _nn(a, b):
    return jnp.dot(a, b, preferred_element_type=f32)


def _nt(a, b):
    return lax.dot_general(a, b, (((1,), (1,)), ((), ())), preferred_element_type=f32)


def _ld(x):
    return pltpu.bitcast(x, bf16)


def _st(x):
    return pltpu.bitcast(x, i32)


def _tree(op, x3):
    n = x3.shape[0]
    while n > 1:
        h = n // 2
        y = op(x3[:h], x3[h:2 * h])
        if n % 2:
            y = jnp.concatenate([op(y[:1], x3[2 * h:]), y[1:]], axis=0) if h > 1 else op(y, x3[2 * h:])
        x3, n = y, h
    return x3[0]


def _red(op, s, chunk=128):
    acc = None
    for c in range(0, s.shape[0], chunk):
        part = _tree(op, s[c:c + chunk].reshape(-1, 8, s.shape[1]))
        acc = part if acc is None else op(acc, part)
    return acc


def _tri():
    ki = lax.broadcasted_iota(i32, (128, 128), 0)
    qi = lax.broadcasted_iota(i32, (128, 128), 1)
    return ki <= qi


def _phi(t):
    return jnp.where(t > 0, t + 1.0, jnp.exp(jnp.minimum(t, 0.0))) + 1e-6


_B_ROWS = [(0, 144), (112, 288), (240, 400), (352, 448)]
_B_TILE = [(0, 128), (128, 256), (256, 384), (384, 448)]


def _kernel(xa_h, ckv_h, wq_h, wk_h, wv_h, wo_h, wqkv_h, wob_h, gw_h, out_ref,
            xa, ckv, wq_raw, wk_raw, wv_raw, wo, wqkv, wob, gw,
            wqkvT, wobT, gvec, kvs, wqT, wk, wvT, qT, kk, vT, oT, acc, sems, *, cfg):
    W, BK, DEPTH, CW = cfg["W"], cfg["BK"], cfg["DEPTH"], cfg["CW"]
    halves = lambda src, dst, s0: [
        pltpu.make_async_copy(src.bitcast(i32).at[:, pl.ds(t * 128, 128)], dst.at[t], sems.at[s0 + t])
        for t in range(2)]
    cps = {
        "wqkv": [pltpu.make_async_copy(wqkv_h, wqkv, sems.at[0])],
        "wob": [pltpu.make_async_copy(wob_h, wob, sems.at[2])],
        "gw": [pltpu.make_async_copy(gw_h, gw, sems.at[3])],
        "xa": [pltpu.make_async_copy(xa_h.bitcast(i32), xa, sems.at[4])],
        "ckv": [pltpu.make_async_copy(ckv_h.bitcast(i32), ckv, sems.at[5])],
        "wq": halves(wq_h, wq_raw, 6),
        "wk": halves(wk_h, wk_raw, 8),
        "wv": halves(wv_h, wv_raw, 10),
        "wo": [pltpu.make_async_copy(wo_h.bitcast(i32), wo, sems.at[12])],
    }
    for name in ("wqkv", "xa", "wob", "gw", "wq", "ckv", "wk", "wv", "wo"):
        for cp in cps[name]:
            cp.start()

    def wait(name):
        for cp in cps[name]:
            cp.wait()

    wait("wqkv")
    for f0 in range(0, 3 * M, 128):
        wdt = min(128, 3 * M - f0)
        blk = wqkv[:, f0:f0 + wdt].astype(f32).T.astype(bf16)
        wqkvT[f0 // 2:(f0 + wdt) // 2, :] = _st(blk)
    wait("wob")
    for f0 in range(0, M, 128):
        wdt = min(128, M - f0)
        wobT[f0 // 2:(f0 + wdt) // 2, :] = _st(wob[:, f0:f0 + wdt].astype(f32).T.astype(bf16))
    wait("xa")

    w_kv = _ld(wqkvT[M // 2:3 * M // 2, :])
    kv_acc = [None] * 4
    for c in range(S // CW):
        xc = _ld(xa[:, c * CW:(c + 1) * CW])
        kvt = _nn(w_kv, xc)
        pk = _phi(kvt[:M]).astype(bf16)
        v = kvt[M:].astype(bf16)
        ones = jnp.ones((16, CW), bf16)
        for j in range(4):
            r0, r1 = _B_ROWS[j]
            d0, d1 = _B_TILE[j]
            lhs = jnp.concatenate([v[r0:r1], ones], axis=0)
            part = _nt(lhs, pk[d0:d1])
            kv_acc[j] = part if kv_acc[j] is None else kv_acc[j] + part
    lhs2 = []
    for j in range(4):
        r0, r1 = _B_ROWS[j]
        d0, d1 = _B_TILE[j]
        n = r1 - r0
        eh = (lax.broadcasted_iota(i32, (n, d1 - d0), 0) + r0) // DH
        dh = (lax.broadcasted_iota(i32, (n, d1 - d0), 1) + d0) // DH
        same = eh == dh
        kvm = jnp.where(same, kv_acc[j][:n], 0.0)
        zm = jnp.where(same, jnp.broadcast_to(kv_acc[j][n:n + 1], (n, d1 - d0)), 0.0)
        lhs2.append(jnp.concatenate([kvm, zm], axis=0).astype(bf16))

    wait("gw")
    gcol = jnp.broadcast_to(gw[...].astype(f32).reshape(1, M), (128, M)).T
    for t in range(NT):
        prod = _ld(xa[:, t * 128:(t + 1) * 128]).astype(f32) * gcol
        z = jnp.sum(prod.reshape(M // 8, 8, 128), axis=0)
        z = jnp.sum(z, axis=0, keepdims=True)
        gvec[:, t * 128:(t + 1) * 128] = jnp.broadcast_to(jax.nn.sigmoid(z), (8, 128))

    w_q = _ld(wqkvT[0:M // 2, :])
    w_ob = _ld(wobT[...])
    for c in range(S // CW):
        xc = _ld(xa[:, c * CW:(c + 1) * CW])
        pq = _phi(_nn(w_q, xc)).astype(bf16)
        nums, dens = [], []
        for j in range(4):
            r0, r1 = _B_ROWS[j]
            d0, d1 = _B_TILE[j]
            r = _nn(lhs2[j], pq[d0:d1])
            nums.append(r[:r1 - r0])
            dens.append(r[r1 - r0:])

        def merge(p):
            return jnp.concatenate([
                p[0][0:112], p[0][112:144] + p[1][0:32], p[1][32:128], p[1][128:176] + p[2][0:48],
                p[2][48:112], p[2][112:160] + p[3][0:48], p[3][48:96]], axis=0)
        num, den = merge(nums), merge(dens)
        g = gvec[0:1, c * CW:(c + 1) * CW]
        o = (num / (den + 1e-6) * (1.0 - g)).astype(bf16)
        acc[:, c * CW:(c + 1) * CW] = _nn(w_ob, o)

    def unpack(w, sh):
        return pltpu.bitcast(lax.shift_left(w, jnp.broadcast_to(sh, w.shape)) & i32(-65536), f32).astype(bf16)

    def relayout_jobs(h):
        j = h // 2
        sh = (1 - h % 2) * 16
        jobs = []
        for dt in range(2):
            for m0 in range(0, M, 128):
                mw = min(128, M - m0)

                def job(dt=dt, m0=m0, mw=mw):
                    w = wq_raw[dt, pl.ds(8 * m0 + j, mw, stride=8), :]
                    wqT[dt * 64:(dt + 1) * 64, m0:m0 + mw] = _st(unpack(w.T, sh))
                jobs.append(job)
        for dt in range(2):
            for c0 in range(0, C, 128):
                def job(dt=dt, c0=c0):
                    w = wk_raw[dt, pl.ds(8 * c0 + j, 128, stride=8), :]
                    wk[c0 // 2:c0 // 2 + 64, dt * 128:(dt + 1) * 128] = _st(unpack(w, sh))
                jobs.append(job)

                def job2(dt=dt, c0=c0):
                    w = wv_raw[dt, pl.ds(8 * c0 + j, 128, stride=8), :]
                    wvT[dt * 64:(dt + 1) * 64, c0:c0 + 128] = _st(unpack(w.T, sh))
                jobs.append(job2)
        return jobs

    wait("wq")
    wait("ckv")
    wait("wk")
    wait("wv")
    for job in relayout_jobs(0):
        job()
    wait("wo")

    def head(h, carry):
        w_qT = _ld(wqT[...])[:, :M]
        for t in range(NT):
            q = _nn(w_qT, _ld(xa[:, t * 128:(t + 1) * 128])) * (D ** -0.5 * LOG2E)
            qT[t] = _st(q.astype(bf16))
        w_k = _ld(wk[...])
        for c in range(S // 256):
            kk[c * 128:(c + 1) * 128, :] = _st(_nn(_ld(ckv[c * 128:(c + 1) * 128, :]), w_k).astype(bf16))
        w_vT = _ld(wvT[...])
        for t in range(NT):
            vT[t] = _st(_nt(w_vT, _ld(ckv[t * 64:(t + 1) * 64, :])).astype(bf16))

        tasks = []
        for qb in range(NT // W):
            q0 = qb * W * 128
            for k0 in range(0, q0, BK):
                tasks.append(("full", qb, k0, min(BK, q0 - k0)))
            for t in range(W):
                tasks.append(("diag", qb, t))
        state = {}

        def tiles(ref, t0, n):
            xs = [_ld(ref[t]) for t in range(t0, t0 + n)]
            return jnp.concatenate(xs, axis=1) if n > 1 else xs[0]

        def do_qk(task):
            if task[0] == "full":
                _, qb, k0, nk = task
                s = _nn(_ld(kk[k0 // 2:(k0 + nk) // 2, :]), tiles(qT, qb * W, W))
            else:
                _, qb, t = task
                q0, nk = qb * W * 128, 128 * (t + 1)
                s = _nn(_ld(kk[q0 // 2:(q0 + nk) // 2, :]), tiles(qT, qb * W + t, 1))
                dg = jnp.where(_tri(), s[nk - 128:], NEG)
                s = jnp.concatenate([s[:nk - 128], dg], axis=0) if nk > 128 else dg
            return s, jnp.max(_red(jnp.maximum, s), axis=0, keepdims=True)

        def upd(st_, s, mx, v):
            if st_ is None:
                p = jnp.exp2(s - mx)
                return mx, _red(jnp.add, p), _nn(v, p.astype(bf16))
            m, l, a = st_
            m_new = jnp.maximum(m, mx)
            alpha = jnp.exp2(m - m_new)
            p = jnp.exp2(s - m_new)
            return m_new, alpha * l + _red(jnp.add, p), a * alpha + _nn(v, p.astype(bf16))

        def do_pv(task, s, mx):
            if task[0] == "full":
                _, qb, k0, nk = task
                state[qb] = upd(state.get(qb), s, mx, tiles(vT, k0 // 128, nk // 128))
                return None
            _, qb, t = task
            full = state.get(qb)
            sl = slice(t * 128, (t + 1) * 128)
            st_ = None if full is None else tuple(x[:, sl] for x in full)
            _, l, a = upd(st_, s, mx, tiles(vT, qb * W, t + 1))
            tt = qb * W + t
            scale = gvec[0:1, tt * 128:(tt + 1) * 128] / jnp.sum(l, axis=0, keepdims=True)
            oT[tt] = _st((a * scale).astype(bf16))
            return tt

        def out_proj(tt):
            w_o = _ld(wo[pl.ds(pl.multiple_of(h * (M // 2), 8), M // 2), :])
            acc[:, tt * 128:(tt + 1) * 128] += _nn(w_o, _ld(oT[tt]))

        jobs = relayout_jobs(jnp.minimum(h + 1, H - 1))
        n = len(tasks)
        per = -(-len(jobs) // n)
        pend, done = [], []
        for i in range(n + DEPTH):
            if i < n:
                pend.append((tasks[i],) + do_qk(tasks[i]))
            if i >= DEPTH:
                tt = do_pv(*pend.pop(0))
                if tt is not None:
                    done.append((i, tt))
            while done and (i - done[0][0] >= cfg["OLAG"]):
                out_proj(done.pop(0)[1])
            for job in jobs[i * per:(i + 1) * per]:
                job()
        for _, tt in done:
            out_proj(tt)
        return carry

    lax.fori_loop(0, H, head, 0)
    out_ref[...] = acc[...].astype(bf16)


CFG = dict(W=1, BK=256, DEPTH=4, CW=512, OLAG=2)


def build(cfg=CFG, name="fused"):
    def run(A_x, A_c_kv, A_w_q, A_w_uk, A_w_uv, A_w_o, B_x, B_wqkv, B_wo, gate_w):
        any_spec = pl.BlockSpec(memory_space=pl.ANY)
        VM = pltpu.VMEM
        outT = pl.pallas_call(
            functools.partial(_kernel, cfg=cfg),
            out_shape=jax.ShapeDtypeStruct((M, S), bf16),
            in_specs=[any_spec] * 9,
            out_specs=pl.BlockSpec(memory_space=pltpu.VMEM),
            scratch_shapes=[
                VM((M // 2, S), i32), VM((S // 2, C), i32),
                VM((2, M * 8, 128), i32), VM((2, C * 8, 128), i32), VM((2, C * 8, 128), i32),
                VM((H * M // 2, D), i32),
                VM((M, 3 * M), bf16), VM((M, M), bf16), VM((M,), bf16),
                VM((3 * M // 2, M), i32), VM((M // 2, M), i32), VM((8, S), f32), VM((8, 128), f32),
                VM((128, 512), i32), VM((C // 2, D), i32), VM((128, C), i32),
                VM((NT, 128, 128), i32), VM((S // 2, D), i32), VM((NT, 128, 128), i32), VM((NT, 128, 128), i32),
                VM((M, S), f32), pltpu.SemaphoreType.DMA((13,)),
            ],
            compiler_params=pltpu.CompilerParams(vmem_limit_bytes=110 * 1024 * 1024),
            name=name,
        )(
            A_x.reshape(S, M).T, A_c_kv.reshape(S, C), A_w_q.reshape(M * H, D),
            A_w_uk.reshape(C * H, D), A_w_uv.reshape(C * H, D),
            jnp.swapaxes(A_w_o, 1, 2).reshape(H * M, D), B_wqkv, B_wo, gate_w,
        )
        return outT.T.reshape(1, S, M)
    return run


@jax.jit
def pallas_gated_mix__compressed_kv_cla__linear_attn_block__prompt_kernel(
        A_x, A_c_kv, A_w_q, A_w_uk, A_w_uv, A_w_o, B_x, B_wqkv, B_wo, gate_w):
    return build()(A_x, A_c_kv, A_w_q, A_w_uk, A_w_uv, A_w_o, B_x, B_wqkv, B_wo, gate_w)
```

```python
import functools
import jax
import jax.numpy as jnp
from jax import lax
import jax.experimental.pallas as pl
import jax.experimental.pallas.tpu as pltpu

S = 2048
M = 448
H = 16
D = 256
C = 1024
DH = 28
NT = S // 128
NEG = -1e30
LOG2E = 1.4426950408889634
f32, bf16, i32 = jnp.float32, jnp.bfloat16, jnp.int32


def _nn(a, b):
    return jnp.dot(a, b, preferred_element_type=f32)


def _nt(a, b):
    return lax.dot_general(a, b, (((1,), (1,)), ((), ())), preferred_element_type=f32)


def _ld(x):
    return pltpu.bitcast(x, bf16)


def _st(x):
    return pltpu.bitcast(x, i32)


def _tree(op, x3):
    n = x3.shape[0]
    while n > 1:
        h = n // 2
        y = op(x3[:h], x3[h:2 * h])
        if n % 2:
            y = jnp.concatenate([op(y[:1], x3[2 * h:]), y[1:]], axis=0) if h > 1 else op(y, x3[2 * h:])
        x3, n = y, h
    return x3[0]


def _red(op, s, chunk=128):
    acc = None
    for c in range(0, s.shape[0], chunk):
        part = _tree(op, s[c:c + chunk].reshape(-1, 8, s.shape[1]))
        acc = part if acc is None else op(acc, part)
    return acc


def _tri():
    ki = lax.broadcasted_iota(i32, (128, 128), 0)
    qi = lax.broadcasted_iota(i32, (128, 128), 1)
    return ki <= qi


def _phi(t):
    return jnp.where(t > 0, t + 1.0, jnp.exp(jnp.minimum(t, 0.0))) + 1e-6


_B_ROWS = [(0, 144), (112, 288), (240, 400), (352, 448)]
_B_TILE = [(0, 128), (128, 256), (256, 384), (384, 448)]


def _kernel(xa_h, ckv_h, wq_h, wk_h, wv_h, wo_h, wqkv_h, wob_h, gw_h, out_h,
            xa, ckv, wq_raw, wk_raw, wv_raw, wo, wqkv, wob, gw,
            wqkvT, wobT, gvec, gcol, kvacc, kvz, wqT, wk, wvT, qT, kk, vT, oT, acc, outs, sems, *, cfg):
    W, BK, DEPTH, CW = cfg["W"], cfg["BK"], cfg["DEPTH"], cfg["CW"]
    halves = lambda src, dst, s0: [
        pltpu.make_async_copy(src.bitcast(i32).at[:, pl.ds(t * 128, 128)], dst.at[t], sems.at[s0 + t])
        for t in range(2)]
    cps = {
        "wqkv": [pltpu.make_async_copy(wqkv_h, wqkv, sems.at[0])],
        "wob": [pltpu.make_async_copy(wob_h, wob, sems.at[2])],
        "gw": [pltpu.make_async_copy(gw_h, gw, sems.at[3])],
        "xa": [pltpu.make_async_copy(xa_h.bitcast(i32), xa, sems.at[4])],
        "ckv": [pltpu.make_async_copy(ckv_h.bitcast(i32), ckv, sems.at[5])],
        "wq": halves(wq_h, wq_raw, 6),
        "wk": halves(wk_h, wk_raw, 8),
        "wv": halves(wv_h, wv_raw, 10),
        "wo": [pltpu.make_async_copy(wo_h.bitcast(i32), wo, sems.at[12])],
    }

    def start(*names):
        for name in names:
            for cp in cps[name]:
                cp.start()

    def wait(*names):
        for name in names:
            for cp in cps[name]:
                cp.wait()

    start("wqkv", "wob", "gw")
    if cfg.get("XA0"):
        start("xa")

    def unpack(w, sh):
        return pltpu.bitcast(lax.shift_left(w, jnp.broadcast_to(sh, w.shape)) & i32(-65536), f32).astype(bf16)

    def wq_jobs(j):
        jobs = []
        for dt in range(2):
            for m0 in range(0, M, 128):
                mw = min(128, M - m0)

                def job(dt=dt, m0=m0, mw=mw):
                    w = wq_raw[dt, pl.ds(8 * m0 + j, mw, stride=8), :].T
                    wqT[dt * 64:(dt + 1) * 64, m0:m0 + mw] = _st(pltpu.bitcast(w << 16, f32).astype(bf16))
                    wqT[128 + dt * 64:128 + (dt + 1) * 64, m0:m0 + mw] = _st(
                        pltpu.bitcast(w & i32(-65536), f32).astype(bf16))
                jobs.append(job)
        return jobs

    def wkv_jobs(h, part=0, nparts=1):
        j = h // 2
        sh = (1 - h % 2) * 16
        jobs = []
        nc = C // 128 // nparts
        for dt in range(2):
            for ci in range(nc):
                cb = part * nc + ci

                def job(dt=dt, cb=cb):
                    w = wk_raw[dt, pl.ds(1024 * cb + j, 128, stride=8), :]
                    wk[pl.ds(pl.multiple_of(cb * 64, 64), 64), dt * 128:(dt + 1) * 128] = _st(unpack(w, sh))
                jobs.append(job)

                def job2(dt=dt, cb=cb):
                    w = wv_raw[dt, pl.ds(1024 * cb + j, 128, stride=8), :]
                    wvT[cb, dt * 64:(dt + 1) * 64, :] = _st(unpack(w.T, sh))
                jobs.append(job2)
        return jobs

    wait("wqkv")
    if not cfg.get("XA0"):
        start("xa")
    for f0 in range(0, 3 * M, 128):
        wdt = min(128, 3 * M - f0)
        wqkvT[f0 // 2:(f0 + wdt) // 2, :] = _st(wqkv[:, f0:f0 + wdt].astype(f32).T.astype(bf16))
    wait("wob", "gw")
    for f0 in range(0, M, 128):
        wdt = min(128, M - f0)
        wobT[f0 // 2:(f0 + wdt) // 2, :] = _st(wob[:, f0:f0 + wdt].astype(f32).T.astype(bf16))
    gcol[...] = jnp.broadcast_to(gw[...].astype(f32).reshape(1, M), (128, M)).T
    kvacc[...] = jnp.zeros(kvacc.shape, f32)
    wait("xa")
    start("wq")
    if cfg.get("ALL1"):
        start("ckv", "wk", "wv", "wo")
    kv_off = [0, 160, 352, 528]
    NSUB = cfg["NSUB"]
    SW = CW // NSUB

    def b1_chunk(i, carry):
        w_kv = _ld(wqkvT[M // 2:3 * M // 2, :])
        pend = []
        for c in range(NSUB + 1):
            if c < NSUB:
                x = _ld(xa[:, pl.ds(pl.multiple_of(i * CW + c * SW, 128), SW)])
                kvt = _nn(w_kv, x)
                pend.append((_phi(kvt[:M]).astype(bf16), kvt[M:].astype(bf16)))
            if c >= 1:
                pk, v = pend.pop(0)
                ones = jnp.ones((16, SW), bf16)
                for j in range(4):
                    r0, r1 = _B_ROWS[j]
                    d0, d1 = _B_TILE[j]
                    part = _nt(jnp.concatenate([v[r0:r1], ones], axis=0), pk[d0:d1])
                    kvacc[kv_off[j]:kv_off[j] + r1 - r0 + 16, 0:d1 - d0] += part
        return carry

    lax.fori_loop(0, S // CW, b1_chunk, 0)
    wait("wq")
    if not cfg.get("ALL1"):
        start("ckv", "wk", "wv", "wo")
    for job in wq_jobs(0):
        job()
    off = 0
    for j in range(4):
        r0, r1 = _B_ROWS[j]
        d0, d1 = _B_TILE[j]
        n = r1 - r0
        eh = (lax.broadcasted_iota(i32, (n, d1 - d0), 0) + r0) // DH
        dh = (lax.broadcasted_iota(i32, (n, d1 - d0), 1) + d0) // DH
        same = eh == dh
        kvj = kvacc[kv_off[j]:kv_off[j] + n + 16, 0:d1 - d0]
        kvm = jnp.where(same, kvj[:n], 0.0)
        hz = lax.broadcasted_iota(i32, (H, d1 - d0), 0) == (lax.broadcasted_iota(i32, (H, d1 - d0), 1) + d0) // DH
        zm = jnp.where(hz, kvj[n:n + H], 0.0)
        kvz[off:off + (n + H) // 2, 0:d1 - d0] = _st(jnp.concatenate([kvm, zm], axis=0).astype(bf16))
        off += (n + H) // 2

    def q_pair(j, carry):
        w = _ld(wqT[...])[:, :M]
        jobs = wq_jobs(jnp.minimum(j + 1, H // 2 - 1))
        for t in range(NT):
            q = _nn(w, _ld(xa[:, t * 128:(t + 1) * 128])) * (D ** -0.5 * LOG2E)
            q = _st(q.astype(bf16))
            qT[2 * j, t] = q[:128]
            qT[2 * j + 1, t] = q[128:]
            if t >= NT - len(jobs):
                jobs[t - (NT - len(jobs))]()
        return carry

    lax.fori_loop(0, H // 2, q_pair, 0)

    wait("ckv", "wk", "wv")

    def merge(p):
        return jnp.concatenate([
            p[0][0:112], p[0][112:144] + p[1][0:32], p[1][32:128], p[1][128:176] + p[2][0:48],
            p[2][48:112], p[2][112:160] + p[3][0:48], p[3][48:96]], axis=0)

    def spread(r16):
        bc = [jnp.broadcast_to(r16[h:h + 1], (8, r16.shape[1])) for h in range(H)]
        low = lax.broadcasted_iota(i32, bc[0].shape, 0) < 4
        rows = []
        for r in range(0, M, 8):
            h0, h1 = r // DH, (r + 7) // DH
            rows.append(bc[h0] if h0 == h1 else jnp.where(low, bc[h0], bc[h1]))
        return jnp.concatenate(rows, axis=0)

    def b2_chunk(i, carry):
        w_q = _ld(wqkvT[0:M // 2, :])
        w_ob = _ld(wobT[...])
        lhs2, off = [], 0
        for j in range(4):
            n = _B_ROWS[j][1] - _B_ROWS[j][0]
            lhs2.append(_ld(kvz[off:off + (n + H) // 2, 0:_B_TILE[j][1] - _B_TILE[j][0]]))
            off += (n + H) // 2
        jobs = wkv_jobs(0, i, S // CW)
        per = -(-len(jobs) // NSUB)
        pa, pb = [], []
        for c in range(NSUB + 2):
            if c < NSUB:
                col = pl.ds(pl.multiple_of(i * CW + c * SW, 128), SW)
                x = _ld(xa[:, col])
                gs = []
                for t in range(SW // 128):
                    prod = x[:, t * 128:(t + 1) * 128].astype(f32) * gcol[...]
                    z = jnp.sum(jnp.sum(prod.reshape(M // 8, 8, 128), axis=0), axis=0, keepdims=True)
                    gs.append(jax.nn.sigmoid(z))
                g = jnp.concatenate(gs, axis=1) if len(gs) > 1 else gs[0]
                gvec[:, col] = jnp.broadcast_to(g, (8, SW))
                pa.append((_phi(_nn(w_q, x)).astype(bf16), g))
                for job in jobs[c * per:(c + 1) * per]:
                    job()
            if 1 <= c <= NSUB:
                pq, g = pa.pop(0)
                nums, dens = [], []
                for j in range(4):
                    n = _B_ROWS[j][1] - _B_ROWS[j][0]
                    d0, d1 = _B_TILE[j]
                    r = _nn(lhs2[j], pq[d0:d1])
                    nums.append(r[:n])
                    dens.append(r[n:])
                r16 = (1.0 - g) / ((dens[0] + dens[1]) + (dens[2] + dens[3]) + 1e-6)
                pb.append((merge(nums) * spread(r16)).astype(bf16))
            if c >= 2:
                acc[:, pl.ds(pl.multiple_of(i * CW + (c - 2) * SW, 128), SW)] = _nn(w_ob, pb.pop(0))
        return carry

    lax.fori_loop(0, S // CW, b2_chunk, 0)
    wait("wo")

    def head(h, carry):
        w_k = _ld(wk[...])
        for c in range(S // 256):
            kk[c * 128:(c + 1) * 128, :] = _st(_nn(_ld(ckv[c * 128:(c + 1) * 128, :]), w_k).astype(bf16))
        w_vT = jnp.concatenate([_ld(wvT[cb]) for cb in range(C // 128)], axis=1)
        for t in range(NT - 1, -1, -1):
            vT[t] = _st(_nt(w_vT, _ld(ckv[t * 64:(t + 1) * 64, :])).astype(bf16))

        tasks = []
        for qb in range(NT // W - 1, -1, -1):
            q0 = qb * W * 128
            for k0 in range(0, q0, BK):
                tasks.append(("full", qb, k0, min(BK, q0 - k0)))
            for t in range(W):
                tasks.append(("diag", qb, t))
        state = {}

        def tiles(get, t0, n):
            xs = [_ld(get(t)) for t in range(t0, t0 + n)]
            return jnp.concatenate(xs, axis=1) if n > 1 else xs[0]
        get_q = lambda t: qT[h, t]
        get_v = lambda t: vT[t]

        def do_qk(task):
            if task[0] == "full":
                _, qb, k0, nk = task
                s = _nn(_ld(kk[k0 // 2:(k0 + nk) // 2, :]), tiles(get_q, qb * W, W))
            else:
                _, qb, t = task
                q0, nk = qb * W * 128, 128 * (t + 1)
                s = _nn(_ld(kk[q0 // 2:(q0 + nk) // 2, :]), tiles(get_q, qb * W + t, 1))
                dg = jnp.where(_tri(), s[nk - 128:], NEG)
                s = jnp.concatenate([s[:nk - 128], dg], axis=0) if nk > 128 else dg
            return s, jnp.max(_red(jnp.maximum, s), axis=0, keepdims=True)

        def upd(st_, s, mx, v):
            if st_ is None:
                p = jnp.exp2(s - mx)
                return mx, _red(jnp.add, p), _nn(v, p.astype(bf16))
            m, l, a = st_
            m_new = jnp.maximum(m, mx)
            alpha = jnp.exp2(m - m_new)
            p = jnp.exp2(s - m_new)
            return m_new, alpha * l + _red(jnp.add, p), a * alpha + _nn(v, p.astype(bf16))

        def do_pv(task, s, mx):
            if task[0] == "full":
                _, qb, k0, nk = task
                state[qb] = upd(state.get(qb), s, mx, tiles(get_v, k0 // 128, nk // 128))
                return None
            _, qb, t = task
            full = state.get(qb)
            sl = slice(t * 128, (t + 1) * 128)
            st_ = None if full is None else tuple(x[:, sl] for x in full)
            _, l, a = upd(st_, s, mx, tiles(get_v, qb * W, t + 1))
            tt = qb * W + t
            scale = gvec[0:1, tt * 128:(tt + 1) * 128] / jnp.sum(l, axis=0, keepdims=True)
            oT[tt] = _st((a * scale).astype(bf16))
            return tt

        def out_proj(tt):
            w_o = _ld(wo[pl.ds(pl.multiple_of(h * (M // 2), 8), M // 2), :])
            acc[:, tt * 128:(tt + 1) * 128] += _nn(w_o, _ld(oT[tt]))

        jobs = wkv_jobs(jnp.minimum(h + 1, H - 1))
        n = len(tasks)
        per = -(-len(jobs) // n)
        pend, done = [], []
        for i in range(n + DEPTH):
            if i < n:
                pend.append((tasks[i],) + do_qk(tasks[i]))
            if i >= DEPTH:
                tt = do_pv(*pend.pop(0))
                if tt is not None:
                    done.append((i, tt))
            while done and (i - done[0][0] >= cfg["OLAG"]):
                out_proj(done.pop(0)[1])
            for job in jobs[i * per:(i + 1) * per]:
                job()
        for _, tt in done:
            out_proj(tt)
        return carry

    lax.fori_loop(0, cfg.get("NH", H), head, 0)

    ocp = []
    NO = 4
    for c in range(NO):
        cw = S // NO
        outs[c] = _st(acc[:, c * cw:(c + 1) * cw].astype(bf16))
        cp = pltpu.make_async_copy(outs.at[c], out_h.bitcast(i32).at[:, pl.ds(c * cw, cw)], sems.at[13 + c])
        cp.start()
        ocp.append(cp)
    for cp in ocp:
        cp.wait()


CFG = dict(W=2, BK=128, DEPTH=6, CW=512, NSUB=2, OLAG=8)


def build(cfg=CFG, name="fused"):
    def run(A_x, A_c_kv, A_w_q, A_w_uk, A_w_uv, A_w_o, B_x, B_wqkv, B_wo, gate_w):
        any_spec = pl.BlockSpec(memory_space=pl.ANY)
        VM = pltpu.VMEM
        outT = pl.pallas_call(
            functools.partial(_kernel, cfg=cfg),
            out_shape=jax.ShapeDtypeStruct((M, S), bf16),
            in_specs=[any_spec] * 9,
            out_specs=any_spec,
            scratch_shapes=[
                VM((M // 2, S), i32), VM((S // 2, C), i32),
                VM((2, M * 8, 128), i32), VM((2, C * 8, 128), i32), VM((2, C * 8, 128), i32),
                VM((H * M // 2, D), i32),
                VM((M, 3 * M), bf16), VM((M, M), bf16), VM((M,), bf16),
                VM((3 * M // 2, M), i32), VM((M // 2, M), i32), VM((8, S), f32), VM((M, 128), f32), VM((640, 128), f32), VM((576, 128), i32),
                VM((256, 512), i32), VM((C // 2, D), i32), VM((C // 128, 128, 128), i32),
                VM((H, NT, 128, 128), i32), VM((S // 2, D), i32), VM((NT, 128, 128), i32), VM((NT, 128, 128), i32),
                VM((M, S), f32), VM((4, M // 2, S // 4), i32), pltpu.SemaphoreType.DMA((17,)),
            ],
            compiler_params=pltpu.CompilerParams(vmem_limit_bytes=110 * 1024 * 1024),
            name=name,
        )(
            A_x.reshape(S, M).T, A_c_kv.reshape(S, C), A_w_q.reshape(M * H, D),
            A_w_uk.reshape(C * H, D), A_w_uv.reshape(C * H, D),
            jnp.swapaxes(A_w_o, 1, 2).reshape(H * M, D), B_wqkv, B_wo, gate_w,
        )
        return outT.T.reshape(1, S, M)
    return run


@jax.jit
def pallas_gated_mix__compressed_kv_cla__linear_attn_block__prompt_kernel(
        A_x, A_c_kv, A_w_q, A_w_uk, A_w_uv, A_w_o, B_x, B_wqkv, B_wo, gate_w):
    return build()(A_x, A_c_kv, A_w_q, A_w_uk, A_w_uv, A_w_o, B_x, B_wqkv, B_wo, gate_w)
```

```python
import functools
import jax
import jax.numpy as jnp
from jax import lax
import jax.experimental.pallas as pl
import jax.experimental.pallas.tpu as pltpu

S = 2048
M = 448
H = 16
D = 256
C = 1024
DH = 28
NT = S // 128
NEG = -1e30
LOG2E = 1.4426950408889634
f32, bf16, i32 = jnp.float32, jnp.bfloat16, jnp.int32


def _nn(a, b):
    return jnp.dot(a, b, preferred_element_type=f32)


def _nt(a, b):
    return lax.dot_general(a, b, (((1,), (1,)), ((), ())), preferred_element_type=f32)


def _ld(x):
    return pltpu.bitcast(x, bf16)


def _st(x):
    return pltpu.bitcast(x, i32)


def _tree(op, x3):
    n = x3.shape[0]
    while n > 1:
        h = n // 2
        y = op(x3[:h], x3[h:2 * h])
        if n % 2:
            y = jnp.concatenate([op(y[:1], x3[2 * h:]), y[1:]], axis=0) if h > 1 else op(y, x3[2 * h:])
        x3, n = y, h
    return x3[0]


def _red(op, s, chunk=128):
    acc = None
    for c in range(0, s.shape[0], chunk):
        part = _tree(op, s[c:c + chunk].reshape(-1, 8, s.shape[1]))
        acc = part if acc is None else op(acc, part)
    return acc


def _tri():
    ki = lax.broadcasted_iota(i32, (128, 128), 0)
    qi = lax.broadcasted_iota(i32, (128, 128), 1)
    return ki <= qi


def _phi(t):
    return jnp.where(t > 0, t + 1.0, jnp.exp(jnp.minimum(t, 0.0))) + 1e-6


def _head_of(f):
    return lax.shift_right_logical(f * 2341, 16)


_B_ROWS = [(0, 144), (112, 288), (240, 400), (352, 448)]
_B_TILE = [(0, 128), (128, 256), (256, 384), (384, 448)]


def _kernel(xa_h, ckv_h, wq_h, wk_h, wv_h, wo_h, wqkv_h, wob_h, gw_h, out_h,
            xa, ckv, wq_raw, wk_raw, wv_raw, wo, wqkv, wsm, wob, gw,
            wqkvT, wsmT, wobT, gcol, kvacc, kvz, wqT, wk, wvT, qT, kk, vT, oT, acc, outs, sems, *, cfg):
    W, BK, DEPTH, CW = cfg["W"], cfg["BK"], cfg["DEPTH"], cfg["CW"]
    halves = lambda src, dst, s0: [
        pltpu.make_async_copy(src.bitcast(i32).at[:, pl.ds(t * 128, 128)], dst.at[t], sems.at[s0 + t])
        for t in range(2)]
    xcw = cfg["CW1"]
    cps = {
        "wqkv_kv": [pltpu.make_async_copy(wqkv_h.at[:, pl.ds(384, 3 * M - 384)], wqkv, sems.at[0])],
        "wqkv_q": [pltpu.make_async_copy(wqkv_h.at[:, pl.ds(0, 384)], wsm, sems.at[1])],
        "wob": [pltpu.make_async_copy(wob_h, wob, sems.at[2])],
        "gw": [pltpu.make_async_copy(gw_h, gw, sems.at[3])],
        "ckv": [pltpu.make_async_copy(ckv_h.bitcast(i32), ckv, sems.at[5])],
        "wq": halves(wq_h, wq_raw, 6),
        "wk": halves(wk_h, wk_raw, 8),
        "wv": halves(wv_h, wv_raw, 10),
        "wo": [pltpu.make_async_copy(wo_h.bitcast(i32), wo, sems.at[12])],
    }

    def xa_copy(i):
        col = pl.ds(pl.multiple_of(i * xcw, 128), xcw)
        return pltpu.make_async_copy(xa_h.bitcast(i32).at[:, col], xa.at[:, col], sems.at[21 + i])

    def start(*names):
        for name in names:
            for cp in cps[name]:
                cp.start()

    def wait(*names):
        for name in names:
            for cp in cps[name]:
                cp.wait()

    start("wqkv_kv")
    xa_copy(0).start()

    def unpack(w, sh):
        return pltpu.bitcast(lax.shift_left(w, jnp.broadcast_to(sh, w.shape)) & i32(-65536), f32).astype(bf16)

    def wq_jobs(j):
        jobs = []
        for dt in range(2):
            for m0 in range(0, M, 128):
                mw = min(128, M - m0)

                def job(dt=dt, m0=m0, mw=mw):
                    w = wq_raw[dt, pl.ds(8 * m0 + j, mw, stride=8), :].T
                    wqT[dt * 64:(dt + 1) * 64, m0:m0 + mw] = _st(pltpu.bitcast(w << 16, f32).astype(bf16))
                    wqT[128 + dt * 64:128 + (dt + 1) * 64, m0:m0 + mw] = _st(
                        pltpu.bitcast(w & i32(-65536), f32).astype(bf16))
                jobs.append(job)
        return jobs

    def wkv_jobs(h, part=0, nparts=1):
        j = h // 2
        sh = (1 - h % 2) * 16
        jobs = []
        nc = C // 128 // nparts
        for dt in range(2):
            for ci in range(nc):
                cb = part * nc + ci

                def job(dt=dt, cb=cb):
                    w = wk_raw[dt, pl.ds(1024 * cb + j, 128, stride=8), :]
                    wk[pl.ds(pl.multiple_of(cb * 64, 64), 64), dt * 128:(dt + 1) * 128] = _st(unpack(w, sh))
                jobs.append(job)

                def job2(dt=dt, cb=cb):
                    w = wv_raw[dt, pl.ds(1024 * cb + j, 128, stride=8), :]
                    wvT[cb, dt * 64:(dt + 1) * 64, :] = _st(unpack(w.T, sh))
                jobs.append(job2)
        return jobs

    wait("wqkv_kv")
    for i in range(1, S // xcw):
        xa_copy(i).start()
    for f0 in range(0, 3 * M - 384, 128):
        wdt = min(128, 3 * M - 384 - f0)
        wqkvT[f0 // 2:(f0 + wdt) // 2, :] = _st(wqkv[:, f0:f0 + wdt].astype(f32).T.astype(bf16))
    kvacc[...] = jnp.zeros(kvacc.shape, f32)
    start("wq", "wqkv_q", "wob", "gw")
    kv_off = [0, 160, 352, 528]
    NSUB = cfg["NSUB"]
    SW = CW // NSUB

    def b1_chunk(i, carry):
        xa_copy(i).wait()
        w_kv = _ld(wqkvT[32:32 + M, :])
        pend = []
        NS1 = xcw // SW
        for c in range(NS1 + 1):
            if c < NS1:
                x = _ld(xa[:, pl.ds(pl.multiple_of(i * xcw + c * SW, 128), SW)])
                kvt = _nn(w_kv, x)
                pend.append((_phi(kvt[:M]).astype(bf16), kvt[M:].astype(bf16)))
            if c >= 1:
                pk, v = pend.pop(0)
                ones = jnp.ones((16, SW), bf16)
                for j in range(4):
                    r0, r1 = _B_ROWS[j]
                    d0, d1 = _B_TILE[j]
                    part = _nt(jnp.concatenate([v[r0:r1], ones], axis=0), pk[d0:d1])
                    kvacc[kv_off[j]:kv_off[j] + r1 - r0 + 16, 0:d1 - d0] += part
        return carry

    lax.fori_loop(0, S // xcw, b1_chunk, 0)
    wait("wq")
    start("ckv", "wk", "wv", "wo")
    wait("wqkv_q", "wob", "gw")
    for job in wq_jobs(0):
        job()
    off = 0
    for j in range(4):
        r0, r1 = _B_ROWS[j]
        d0, d1 = _B_TILE[j]
        n = r1 - r0
        eh = _head_of(lax.broadcasted_iota(i32, (n, d1 - d0), 0) + r0)
        dh = _head_of(lax.broadcasted_iota(i32, (n, d1 - d0), 1) + d0)
        same = eh == dh
        kvj = kvacc[kv_off[j]:kv_off[j] + n + 16, 0:d1 - d0]
        kvm = jnp.where(same, kvj[:n], 0.0)
        hz = lax.broadcasted_iota(i32, (H, d1 - d0), 0) == _head_of(lax.broadcasted_iota(i32, (H, d1 - d0), 1) + d0)
        zm = jnp.where(hz, kvj[n:n + H], 0.0)
        kvz[off:off + (n + H) // 2, 0:d1 - d0] = _st(jnp.concatenate([kvm, zm], axis=0).astype(bf16))
        off += (n + H) // 2

    def q_pair(j, carry):
        w = _ld(wqT[:, :M])
        jobs = wq_jobs(jnp.minimum(j + 1, H // 2 - 1))
        jc = jnp.minimum(j, 2)
        rows, cols = pl.ds(pl.multiple_of(jc * 64, 64), 64), pl.ds(pl.multiple_of(jc * 128, 128), 128)
        wsmT[rows, :] = _st(wsm[:, cols].astype(f32).T.astype(bf16))
        wobT[rows, :] = _st(wob[:, cols].astype(f32).T.astype(bf16))
        wobT[192:224, :] = _st(wob[:, 384:M].astype(f32).T.astype(bf16))
        acc[:, pl.ds(pl.multiple_of(j * 256, 256), 256)] = jnp.zeros((M, 256), f32)
        gcol[...] = jnp.broadcast_to(gw[...].astype(f32).reshape(1, M), (128, M)).T
        for t in range(NT):
            q = _nn(w, _ld(xa[:, t * 128:(t + 1) * 128])) * (D ** -0.5 * LOG2E)
            q = _st(q.astype(bf16))
            qT[2 * j, t] = q[:128]
            qT[2 * j + 1, t] = q[128:]
            if t >= NT - len(jobs):
                jobs[t - (NT - len(jobs))]()
        return carry

    lax.fori_loop(0, H // 2, q_pair, 0)

    wait("ckv", "wk", "wv")
    for job in wkv_jobs(0):
        job()
    wait("wo")

    def head(h, carry):
        w_k = _ld(wk[...])
        for c in range(S // 256):
            kk[c * 128:(c + 1) * 128, :] = _st(_nn(_ld(ckv[c * 128:(c + 1) * 128, :]), w_k).astype(bf16))
        w_vT = jnp.concatenate([_ld(wvT[cb]) for cb in range(C // 128)], axis=1)
        for t in range(NT - 1, -1, -1):
            vT[t] = _st(_nt(w_vT, _ld(ckv[t * 64:(t + 1) * 64, :])).astype(bf16))

        tasks = []
        for qb in range(NT // W - 1, -1, -1):
            q0 = qb * W * 128
            for k0 in range(0, q0, BK):
                tasks.append(("full", qb, k0, min(BK, q0 - k0)))
            for t in range(W):
                tasks.append(("diag", qb, t))
        state = {}

        def tiles(get, t0, n):
            xs = [_ld(get(t)) for t in range(t0, t0 + n)]
            return jnp.concatenate(xs, axis=1) if n > 1 else xs[0]
        get_q = lambda t: qT[h, t]
        get_v = lambda t: vT[t]

        def do_qk(task):
            if task[0] == "full":
                _, qb, k0, nk = task
                s = _nn(_ld(kk[k0 // 2:(k0 + nk) // 2, :]), tiles(get_q, qb * W, W))
            else:
                _, qb, t = task
                q0, nk = qb * W * 128, 128 * (t + 1)
                s = _nn(_ld(kk[q0 // 2:(q0 + nk) // 2, :]), tiles(get_q, qb * W + t, 1))
                dg = jnp.where(_tri(), s[nk - 128:], NEG)
                s = jnp.concatenate([s[:nk - 128], dg], axis=0) if nk > 128 else dg
            return s, jnp.max(_red(jnp.maximum, s), axis=0, keepdims=True)

        def upd(st_, s, mx, v):
            if st_ is None:
                p = jnp.exp2(s - mx)
                return mx, _red(jnp.add, p), _nn(v, p.astype(bf16))
            m, l, a = st_
            m_new = jnp.maximum(m, mx)
            alpha = jnp.exp2(m - m_new)
            p = jnp.exp2(s - m_new)
            return m_new, alpha * l + _red(jnp.add, p), a * alpha + _nn(v, p.astype(bf16))

        def do_pv(task, s, mx):
            if task[0] == "full":
                _, qb, k0, nk = task
                state[qb] = upd(state.get(qb), s, mx, tiles(get_v, k0 // 128, nk // 128))
                return None
            _, qb, t = task
            full = state.get(qb)
            sl = slice(t * 128, (t + 1) * 128)
            st_ = None if full is None else tuple(x[:, sl] for x in full)
            _, l, a = upd(st_, s, mx, tiles(get_v, qb * W, t + 1))
            tt = qb * W + t
            scale = 1.0 / jnp.sum(l, axis=0, keepdims=True)
            oT[tt] = _st((a * scale).astype(bf16))
            return tt

        def out_proj(tt):
            w_o = _ld(wo[pl.ds(pl.multiple_of(h * (M // 2), 8), M // 2), :])
            acc[:, tt * 128:(tt + 1) * 128] += _nn(w_o, _ld(oT[tt]))

        jobs = wkv_jobs(jnp.minimum(h + 1, H - 1))
        n = len(tasks)
        per = -(-len(jobs) // n)
        pend, done = [], []
        for i in range(n + DEPTH):
            if i < n:
                pend.append((tasks[i],) + do_qk(tasks[i]))
            if i >= DEPTH:
                tt = do_pv(*pend.pop(0))
                if tt is not None:
                    done.append((i, tt))
            while done and (i - done[0][0] >= cfg["OLAG"]):
                out_proj(done.pop(0)[1])
            for job in jobs[i * per:(i + 1) * per]:
                job()
        for _, tt in done:
            out_proj(tt)
        return carry

    lax.fori_loop(0, H, head, 0)


    def merge(p):
        return jnp.concatenate([
            p[0][0:112], p[0][112:144] + p[1][0:32], p[1][32:128], p[1][128:176] + p[2][0:48],
            p[2][48:112], p[2][112:160] + p[3][0:48], p[3][48:96]], axis=0)

    def spread(r16):
        bc = [jnp.broadcast_to(r16[h:h + 1], (8, r16.shape[1])) for h in range(H)]
        low = lax.broadcasted_iota(i32, bc[0].shape, 0) < 4
        rows = []
        for r in range(0, M, 8):
            h0, h1 = r // DH, (r + 7) // DH
            rows.append(bc[h0] if h0 == h1 else jnp.where(low, bc[h0], bc[h1]))
        return jnp.concatenate(rows, axis=0)

    def out_copy(slot):
        col = pl.ds(pl.multiple_of(slot * SW, 128), SW)
        return pltpu.make_async_copy(outs.at[slot], out_h.bitcast(i32).at[:, col], sems.at[25 + slot])

    def b2_chunk(i, carry):
        w_q = jnp.concatenate([_ld(wsmT[...]), _ld(wqkvT[0:32, :])], axis=0)
        w_ob = _ld(wobT[...])
        lhs2, off = [], 0
        for j in range(4):
            n = _B_ROWS[j][1] - _B_ROWS[j][0]
            lhs2.append(_ld(kvz[off:off + (n + H) // 2, 0:_B_TILE[j][1] - _B_TILE[j][0]]))
            off += (n + H) // 2
        pa, pb = [], []
        for c in range(NSUB + 2):
            if c < NSUB:
                col = pl.ds(pl.multiple_of(i * CW + c * SW, 128), SW)
                x = _ld(xa[:, col])
                gs = []
                for t in range(SW // 128):
                    prod = x[:, t * 128:(t + 1) * 128].astype(f32) * gcol[...]
                    z = jnp.sum(jnp.sum(prod.reshape(M // 8, 8, 128), axis=0), axis=0, keepdims=True)
                    gs.append(jax.nn.sigmoid(z))
                g = jnp.concatenate(gs, axis=1) if len(gs) > 1 else gs[0]
                pa.append((_phi(_nn(w_q, x)).astype(bf16), g))
            if 1 <= c <= NSUB:
                pq, g = pa.pop(0)
                nums, dens = [], []
                for j in range(4):
                    n = _B_ROWS[j][1] - _B_ROWS[j][0]
                    d0, d1 = _B_TILE[j]
                    r = _nn(lhs2[j], pq[d0:d1])
                    nums.append(r[:n])
                    dens.append(r[n:])
                r16 = (1.0 - g) / ((dens[0] + dens[1]) + (dens[2] + dens[3]) + 1e-6)
                pb.append(((merge(nums) * spread(r16)).astype(bf16), g))
            if c >= 2:
                o, g = pb.pop(0)
                col = pl.ds(pl.multiple_of(i * CW + (c - 2) * SW, 128), SW)
                res = g * acc[:, col] + _nn(w_ob, o)
                slot = i * NSUB + c - 2
                outs[slot] = _st(res.astype(bf16))
                out_copy(slot).start()
        return carry

    lax.fori_loop(0, S // CW, b2_chunk, 0)

    for slot in range(S // SW):
        out_copy(slot).wait()


CFG = dict(W=2, BK=128, DEPTH=6, CW=512, NSUB=2, OLAG=8, CW1=512)


def build(cfg=CFG, name="fused"):
    def run(A_x, A_c_kv, A_w_q, A_w_uk, A_w_uv, A_w_o, B_x, B_wqkv, B_wo, gate_w):
        any_spec = pl.BlockSpec(memory_space=pl.ANY)
        VM = pltpu.VMEM
        outT = pl.pallas_call(
            functools.partial(_kernel, cfg=cfg),
            out_shape=jax.ShapeDtypeStruct((M, S), bf16),
            in_specs=[any_spec] * 9,
            out_specs=any_spec,
            scratch_shapes=[
                VM((M // 2, S), i32), VM((S // 2, C), i32),
                VM((2, M * 8, 128), i32), VM((2, C * 8, 128), i32), VM((2, C * 8, 128), i32),
                VM((H * M // 2, D), i32),
                VM((M, 3 * M - 384), bf16), VM((M, 384), bf16), VM((M, M), bf16), VM((M,), bf16),
                VM(((3 * M - 384) // 2, M), i32), VM((192, M), i32), VM((M // 2, M), i32), VM((M, 128), f32), VM((640, 128), f32), VM((576, 128), i32),
                VM((256, 512), i32), VM((C // 2, D), i32), VM((C // 128, 128, 128), i32),
                VM((H, NT, 128, 128), i32), VM((S // 2, D), i32), VM((NT, 128, 128), i32), VM((NT, 128, 128), i32),
                VM((M, S), f32), VM((S * cfg['NSUB'] // cfg['CW'], M // 2, cfg['CW'] // cfg['NSUB']), i32), pltpu.SemaphoreType.DMA((33,)),
            ],
            compiler_params=pltpu.CompilerParams(vmem_limit_bytes=110 * 1024 * 1024),
            name=name,
        )(
            A_x.reshape(S, M).T, A_c_kv.reshape(S, C), A_w_q.reshape(M * H, D),
            A_w_uk.reshape(C * H, D), A_w_uv.reshape(C * H, D),
            jnp.swapaxes(A_w_o, 1, 2).reshape(H * M, D), B_wqkv, B_wo, gate_w,
        )
        return outT.T.reshape(1, S, M)
    return run


@jax.jit
def pallas_gated_mix__compressed_kv_cla__linear_attn_block__prompt_kernel(
        A_x, A_c_kv, A_w_q, A_w_uk, A_w_uv, A_w_o, B_x, B_wqkv, B_wo, gate_w):
    return build()(A_x, A_c_kv, A_w_q, A_w_uk, A_w_uv, A_w_o, B_x, B_wqkv, B_wo, gate_w)
```

```python
import functools
import jax
import jax.numpy as jnp
import numpy as np
from jax import lax
import jax.experimental.pallas as pl
import jax.experimental.pallas.tpu as pltpu

S = 2048
M = 448
H = 16
D = 256
C = 1024
DH = 28
NT = S // 128
NEG = -1e30
LOG2E = 1.4426950408889634
f32, bf16, i32 = jnp.float32, jnp.bfloat16, jnp.int32
_HI_MASK = np.int32(-65536)


def _nn(a, b):
    return jnp.dot(a, b, preferred_element_type=f32)


def _nt(a, b):
    return lax.dot_general(a, b, (((1,), (1,)), ((), ())), preferred_element_type=f32)


def _ld(x):
    return pltpu.bitcast(x, bf16)


def _st(x):
    return pltpu.bitcast(x, i32)


def _tree(op, x3):
    n = x3.shape[0]
    while n > 1:
        h = n // 2
        y = op(x3[:h], x3[h:2 * h])
        if n % 2:
            y = jnp.concatenate([op(y[:1], x3[2 * h:]), y[1:]], axis=0) if h > 1 else op(y, x3[2 * h:])
        x3, n = y, h
    return x3[0]


def _red(op, s, chunk=128):
    acc = None
    for c in range(0, s.shape[0], chunk):
        part = _tree(op, s[c:c + chunk].reshape(-1, 8, s.shape[1]))
        acc = part if acc is None else op(acc, part)
    return acc


def _tri():
    ki = lax.broadcasted_iota(i32, (128, 128), 0)
    qi = lax.broadcasted_iota(i32, (128, 128), 1)
    return ki <= qi


def _phi(t):
    return jnp.where(t > 0, t + 1.0, jnp.exp(jnp.minimum(t, 0.0))) + 1e-6


def _head_of(f):
    return lax.shift_right_logical(f * 2341, 16)


_B_ROWS = [(0, 144), (112, 288), (240, 400), (352, 448)]
_B_TILE = [(0, 128), (128, 256), (256, 384), (384, 448)]


def _kernel(xa_h, ckv_h, wq_h, wk_h, wv_h, wo_h, wqkv_h, wob_h, gw_h, out_h,
            xa, ckv, wq_raw, wk_raw, wv_raw, wo, wqkv, wsm, wob, gw,
            wqkvT, wsmT, wobT, gcol, kvacc, kvz, wqT, wk, wvT, qT, kk, vT, oT, acc, outs, sems, *, cfg):
    W, BK, DEPTH, CW = cfg["W"], cfg["BK"], cfg["DEPTH"], cfg["CW"]
    halves = lambda src, dst, s0: [
        pltpu.make_async_copy(src.bitcast(i32).at[:, pl.ds(t * 128, 128)], dst.at[t], sems.at[s0 + t])
        for t in range(2)]
    xcw = cfg["CW1"]
    cps = {
        "wqkv_kv": [pltpu.make_async_copy(wqkv_h.at[:, pl.ds(384, 3 * M - 384)], wqkv, sems.at[0])],
        "wqkv_q": [pltpu.make_async_copy(wqkv_h.at[:, pl.ds(0, 384)], wsm, sems.at[1])],
        "wob": [pltpu.make_async_copy(wob_h, wob, sems.at[2])],
        "gw": [pltpu.make_async_copy(gw_h, gw, sems.at[3])],
        "ckv": [pltpu.make_async_copy(ckv_h.bitcast(i32), ckv, sems.at[5])],
        "wq": halves(wq_h, wq_raw, 6),
        "wk": halves(wk_h, wk_raw, 8),
        "wv": halves(wv_h, wv_raw, 10),
        "wo": [pltpu.make_async_copy(wo_h.bitcast(i32), wo, sems.at[12])],
    }

    def xa_copy(i):
        col = pl.ds(pl.multiple_of(i * xcw, 128), xcw)
        return pltpu.make_async_copy(xa_h.bitcast(i32).at[:, col], xa.at[:, col], sems.at[21 + i])

    def start(*names):
        for name in names:
            for cp in cps[name]:
                cp.start()

    def wait(*names):
        for name in names:
            for cp in cps[name]:
                cp.wait()

    start("wqkv_kv")
    xa_copy(0).start()

    def unpack(w, sh):
        return pltpu.bitcast(lax.shift_left(w, jnp.broadcast_to(sh, w.shape)) & _HI_MASK, f32).astype(bf16)

    def wq_jobs(j):
        jobs = []
        for dt in range(2):
            for m0 in range(0, M, 128):
                mw = min(128, M - m0)

                def job(dt=dt, m0=m0, mw=mw):
                    w = wq_raw[dt, pl.ds(8 * m0 + j, mw, stride=8), :].T
                    wqT[dt * 64:(dt + 1) * 64, m0:m0 + mw] = _st(pltpu.bitcast(w << 16, f32).astype(bf16))
                    wqT[128 + dt * 64:128 + (dt + 1) * 64, m0:m0 + mw] = _st(
                        pltpu.bitcast(w & _HI_MASK, f32).astype(bf16))
                jobs.append(job)
        return jobs

    def wkv_jobs(h):
        j = h // 2
        sh = (1 - h % 2) * 16
        jobs = []
        for dt in range(2):
            for cb in range(C // 128):
                def job(dt=dt, cb=cb):
                    w = wk_raw[dt, pl.ds(1024 * cb + j, 128, stride=8), :]
                    wk[cb * 64:(cb + 1) * 64, dt * 128:(dt + 1) * 128] = _st(unpack(w, sh))
                jobs.append(job)

                def job2(dt=dt, cb=cb):
                    w = wv_raw[dt, pl.ds(1024 * cb + j, 128, stride=8), :]
                    wvT[cb, dt * 64:(dt + 1) * 64, :] = _st(unpack(w.T, sh))
                jobs.append(job2)
        return jobs

    wait("wqkv_kv")
    for i in range(1, S // xcw):
        xa_copy(i).start()
    for f0 in range(0, 3 * M - 384, 128):
        wdt = min(128, 3 * M - 384 - f0)
        wqkvT[f0 // 2:(f0 + wdt) // 2, :] = _st(wqkv[:, f0:f0 + wdt].astype(f32).T.astype(bf16))
    kvacc[...] = jnp.zeros(kvacc.shape, f32)
    start("wq", "wqkv_q", "wob", "gw")
    kv_off = [0, 160, 352, 528]
    NSUB = cfg["NSUB"]
    SW = CW // NSUB

    def b1_chunk(i, carry):
        xa_copy(i).wait()
        w_kv = _ld(wqkvT[32:32 + M, :])
        pend = []
        NS1 = xcw // SW
        for c in range(NS1 + 1):
            if c < NS1:
                x = _ld(xa[:, pl.ds(pl.multiple_of(i * xcw + c * SW, 128), SW)])
                kvt = _nn(w_kv, x)
                pend.append((_phi(kvt[:M]).astype(bf16), kvt[M:].astype(bf16)))
            if c >= 1:
                pk, v = pend.pop(0)
                ones = jnp.ones((16, SW), bf16)
                for j in range(4):
                    r0, r1 = _B_ROWS[j]
                    d0, d1 = _B_TILE[j]
                    part = _nt(jnp.concatenate([v[r0:r1], ones], axis=0), pk[d0:d1])
                    kvacc[kv_off[j]:kv_off[j] + r1 - r0 + 16, 0:d1 - d0] += part
        return carry

    lax.fori_loop(0, S // xcw, b1_chunk, 0)
    wait("wq")
    start("ckv", "wk", "wv", "wo")
    wait("wqkv_q", "wob", "gw")
    for job in wq_jobs(0):
        job()
    off = 0
    for j in range(4):
        r0, r1 = _B_ROWS[j]
        d0, d1 = _B_TILE[j]
        n = r1 - r0
        eh = _head_of(lax.broadcasted_iota(i32, (n, d1 - d0), 0) + r0)
        dh = _head_of(lax.broadcasted_iota(i32, (n, d1 - d0), 1) + d0)
        same = eh == dh
        kvj = kvacc[kv_off[j]:kv_off[j] + n + 16, 0:d1 - d0]
        kvm = jnp.where(same, kvj[:n], 0.0)
        hz = lax.broadcasted_iota(i32, (H, d1 - d0), 0) == _head_of(lax.broadcasted_iota(i32, (H, d1 - d0), 1) + d0)
        zm = jnp.where(hz, kvj[n:n + H], 0.0)
        kvz[off:off + (n + H) // 2, 0:d1 - d0] = _st(jnp.concatenate([kvm, zm], axis=0).astype(bf16))
        off += (n + H) // 2

    def q_pair(j, carry):
        w = _ld(wqT[:, :M])
        jobs = wq_jobs(jnp.minimum(j + 1, H // 2 - 1))
        jc = jnp.minimum(j, 2)
        rows, cols = pl.ds(pl.multiple_of(jc * 64, 64), 64), pl.ds(pl.multiple_of(jc * 128, 128), 128)
        wsmT[rows, :] = _st(wsm[:, cols].astype(f32).T.astype(bf16))
        wobT[rows, :] = _st(wob[:, cols].astype(f32).T.astype(bf16))
        wobT[192:224, :] = _st(wob[:, 384:M].astype(f32).T.astype(bf16))
        acc[:, pl.ds(pl.multiple_of(j * 256, 256), 256)] = jnp.zeros((M, 256), f32)
        gcol[...] = jnp.broadcast_to(gw[...].astype(f32).reshape(1, M), (128, M)).T
        for t in range(NT):
            q = _nn(w, _ld(xa[:, t * 128:(t + 1) * 128])) * (D ** -0.5 * LOG2E)
            q = _st(q.astype(bf16))
            qT[2 * j, t] = q[:128]
            qT[2 * j + 1, t] = q[128:]
            if t >= NT - len(jobs):
                jobs[t - (NT - len(jobs))]()
        return carry

    lax.fori_loop(0, H // 2, q_pair, 0)

    wait("ckv", "wk", "wv")
    for job in wkv_jobs(0):
        job()
    wait("wo")

    def head(h, carry):
        w_k = _ld(wk[...])
        for c in range(S // 256):
            kk[c * 128:(c + 1) * 128, :] = _st(_nn(_ld(ckv[c * 128:(c + 1) * 128, :]), w_k).astype(bf16))
        w_vT = jnp.concatenate([_ld(wvT[cb]) for cb in range(C // 128)], axis=1)
        for t in range(NT - 1, -1, -1):
            vT[t] = _st(_nt(w_vT, _ld(ckv[t * 64:(t + 1) * 64, :])).astype(bf16))

        tasks = []
        for qb in range(NT // W - 1, -1, -1):
            q0 = qb * W * 128
            for k0 in range(0, q0, BK):
                tasks.append(("full", qb, k0, min(BK, q0 - k0)))
            for t in range(W):
                tasks.append(("diag", qb, t))
        state = {}

        def tiles(get, t0, n):
            xs = [_ld(get(t)) for t in range(t0, t0 + n)]
            return jnp.concatenate(xs, axis=1) if n > 1 else xs[0]
        get_q = lambda t: qT[h, t]
        get_v = lambda t: vT[t]

        def do_qk(task):
            if task[0] == "full":
                _, qb, k0, nk = task
                s = _nn(_ld(kk[k0 // 2:(k0 + nk) // 2, :]), tiles(get_q, qb * W, W))
            else:
                _, qb, t = task
                q0, nk = qb * W * 128, 128 * (t + 1)
                s = _nn(_ld(kk[q0 // 2:(q0 + nk) // 2, :]), tiles(get_q, qb * W + t, 1))
                dg = jnp.where(_tri(), s[nk - 128:], NEG)
                s = jnp.concatenate([s[:nk - 128], dg], axis=0) if nk > 128 else dg
            return s, jnp.max(_red(jnp.maximum, s), axis=0, keepdims=True)

        def upd(st_, s, mx, v):
            if st_ is None:
                p = jnp.exp2(s - mx)
                return mx, _red(jnp.add, p), _nn(v, p.astype(bf16))
            m, l, a = st_
            m_new = jnp.maximum(m, mx)
            alpha = jnp.exp2(m - m_new)
            p = jnp.exp2(s - m_new)
            return m_new, alpha * l + _red(jnp.add, p), a * alpha + _nn(v, p.astype(bf16))

        def do_pv(task, s, mx):
            if task[0] == "full":
                _, qb, k0, nk = task
                state[qb] = upd(state.get(qb), s, mx, tiles(get_v, k0 // 128, nk // 128))
                return None
            _, qb, t = task
            full = state.get(qb)
            sl = slice(t * 128, (t + 1) * 128)
            st_ = None if full is None else tuple(x[:, sl] for x in full)
            _, l, a = upd(st_, s, mx, tiles(get_v, qb * W, t + 1))
            tt = qb * W + t
            scale = 1.0 / jnp.sum(l, axis=0, keepdims=True)
            oT[tt] = _st((a * scale).astype(bf16))
            return tt

        def out_proj(tt):
            w_o = _ld(wo[pl.ds(pl.multiple_of(h * (M // 2), 8), M // 2), :])
            acc[:, tt * 128:(tt + 1) * 128] += _nn(w_o, _ld(oT[tt]))

        jobs = wkv_jobs(jnp.minimum(h + 1, H - 1))
        n = len(tasks)
        per = -(-len(jobs) // n)
        pend, done = [], []
        for i in range(n + DEPTH):
            if i < n:
                pend.append((tasks[i],) + do_qk(tasks[i]))
            if i >= DEPTH:
                tt = do_pv(*pend.pop(0))
                if tt is not None:
                    done.append((i, tt))
            while done and (i - done[0][0] >= cfg["OLAG"]):
                out_proj(done.pop(0)[1])
            for job in jobs[i * per:(i + 1) * per]:
                job()
        for _, tt in done:
            out_proj(tt)
        return carry

    lax.fori_loop(0, H, head, 0)


    def merge(p):
        return jnp.concatenate([
            p[0][0:112], p[0][112:144] + p[1][0:32], p[1][32:128], p[1][128:176] + p[2][0:48],
            p[2][48:112], p[2][112:160] + p[3][0:48], p[3][48:96]], axis=0)

    def spread(r16):
        bc = [jnp.broadcast_to(r16[h:h + 1], (8, r16.shape[1])) for h in range(H)]
        low = lax.broadcasted_iota(i32, bc[0].shape, 0) < 4
        rows = []
        for r in range(0, M, 8):
            h0, h1 = r // DH, (r + 7) // DH
            rows.append(bc[h0] if h0 == h1 else jnp.where(low, bc[h0], bc[h1]))
        return jnp.concatenate(rows, axis=0)

    def out_copy(slot):
        col = pl.ds(pl.multiple_of(slot * SW, 128), SW)
        return pltpu.make_async_copy(outs.at[slot], out_h.bitcast(i32).at[:, col], sems.at[25 + slot])

    def b2_chunk(i, carry):
        w_q = jnp.concatenate([_ld(wsmT[...]), _ld(wqkvT[0:32, :])], axis=0)
        w_ob = _ld(wobT[...])
        lhs2, off = [], 0
        for j in range(4):
            n = _B_ROWS[j][1] - _B_ROWS[j][0]
            lhs2.append(_ld(kvz[off:off + (n + H) // 2, 0:_B_TILE[j][1] - _B_TILE[j][0]]))
            off += (n + H) // 2
        pa, pb = [], []
        for c in range(NSUB + 2):
            if c < NSUB:
                col = pl.ds(pl.multiple_of(i * CW + c * SW, 128), SW)
                x = _ld(xa[:, col])
                gs = []
                for t in range(SW // 128):
                    prod = x[:, t * 128:(t + 1) * 128].astype(f32) * gcol[...]
                    z = jnp.sum(jnp.sum(prod.reshape(M // 8, 8, 128), axis=0), axis=0, keepdims=True)
                    gs.append(jax.nn.sigmoid(z))
                g = jnp.concatenate(gs, axis=1) if len(gs) > 1 else gs[0]
                pa.append((_phi(_nn(w_q, x)).astype(bf16), g))
            if 1 <= c <= NSUB:
                pq, g = pa.pop(0)
                nums, dens = [], []
                for j in range(4):
                    n = _B_ROWS[j][1] - _B_ROWS[j][0]
                    d0, d1 = _B_TILE[j]
                    r = _nn(lhs2[j], pq[d0:d1])
                    nums.append(r[:n])
                    dens.append(r[n:])
                r16 = (1.0 - g) / ((dens[0] + dens[1]) + (dens[2] + dens[3]) + 1e-6)
                pb.append(((merge(nums) * spread(r16)).astype(bf16), g))
            if c >= 2:
                o, g = pb.pop(0)
                col = pl.ds(pl.multiple_of(i * CW + (c - 2) * SW, 128), SW)
                res = g * acc[:, col] + _nn(w_ob, o)
                slot = i * NSUB + c - 2
                outs[slot] = _st(res.astype(bf16))
                out_copy(slot).start()
        return carry

    lax.fori_loop(0, S // CW, b2_chunk, 0)

    for slot in range(S // SW):
        out_copy(slot).wait()


CFG = dict(W=2, BK=128, DEPTH=6, CW=512, NSUB=2, OLAG=8, CW1=512)


def build(cfg=CFG, name="fused"):
    def run(A_x, A_c_kv, A_w_q, A_w_uk, A_w_uv, A_w_o, B_x, B_wqkv, B_wo, gate_w):
        any_spec = pl.BlockSpec(memory_space=pl.ANY)
        VM = pltpu.VMEM
        outT = pl.pallas_call(
            functools.partial(_kernel, cfg=cfg),
            out_shape=jax.ShapeDtypeStruct((M, S), bf16),
            in_specs=[any_spec] * 9,
            out_specs=any_spec,
            scratch_shapes=[
                VM((M // 2, S), i32), VM((S // 2, C), i32),
                VM((2, M * 8, 128), i32), VM((2, C * 8, 128), i32), VM((2, C * 8, 128), i32),
                VM((H * M // 2, D), i32),
                VM((M, 3 * M - 384), bf16), VM((M, 384), bf16), VM((M, M), bf16), VM((M,), bf16),
                VM(((3 * M - 384) // 2, M), i32), VM((192, M), i32), VM((M // 2, M), i32), VM((M, 128), f32), VM((640, 128), f32), VM((576, 128), i32),
                VM((256, 512), i32), VM((C // 2, D), i32), VM((C // 128, 128, 128), i32),
                VM((H, NT, 128, 128), i32), VM((S // 2, D), i32), VM((NT, 128, 128), i32), VM((NT, 128, 128), i32),
                VM((M, S), f32), VM((S * cfg['NSUB'] // cfg['CW'], M // 2, cfg['CW'] // cfg['NSUB']), i32), pltpu.SemaphoreType.DMA((33,)),
            ],
            compiler_params=pltpu.CompilerParams(vmem_limit_bytes=110 * 1024 * 1024),
            name=name,
        )(
            A_x.reshape(S, M).T, A_c_kv.reshape(S, C), A_w_q.reshape(M * H, D),
            A_w_uk.reshape(C * H, D), A_w_uv.reshape(C * H, D),
            jnp.swapaxes(A_w_o, 1, 2).reshape(H * M, D), B_wqkv, B_wo, gate_w,
        )
        return outT.T.reshape(1, S, M)
    return run


@jax.jit
def pallas_gated_mix__compressed_kv_cla__linear_attn_block__prompt_kernel(
        A_x, A_c_kv, A_w_q, A_w_uk, A_w_uv, A_w_o, B_x, B_wqkv, B_wo, gate_w):
    return build()(A_x, A_c_kv, A_w_q, A_w_uk, A_w_uv, A_w_o, B_x, B_wqkv, B_wo, gate_w)
```

```python
import functools
import jax
import jax.numpy as jnp
import numpy as np
from jax import lax
import jax.experimental.pallas as pl
import jax.experimental.pallas.tpu as pltpu

S = 2048
M = 448
H = 16
D = 256
C = 1024
DH = 28
NT = S // 128
NEG = -1e30
LOG2E = 1.4426950408889634
f32, bf16, i32 = jnp.float32, jnp.bfloat16, jnp.int32
_HI_MASK = np.int32(-65536)


def _nn(a, b):
    return jnp.dot(a, b, preferred_element_type=f32)


def _nt(a, b):
    return lax.dot_general(a, b, (((1,), (1,)), ((), ())), preferred_element_type=f32)


def _ld(x):
    return pltpu.bitcast(x, bf16)


def _st(x):
    return pltpu.bitcast(x, i32)


def _tree(op, x3):
    n = x3.shape[0]
    while n > 1:
        h = n // 2
        y = op(x3[:h], x3[h:2 * h])
        if n % 2:
            y = jnp.concatenate([op(y[:1], x3[2 * h:]), y[1:]], axis=0) if h > 1 else op(y, x3[2 * h:])
        x3, n = y, h
    return x3[0]


def _red(op, s, chunk=128):
    acc = None
    for c in range(0, s.shape[0], chunk):
        part = _tree(op, s[c:c + chunk].reshape(-1, 8, s.shape[1]))
        acc = part if acc is None else op(acc, part)
    return acc


def _tri():
    ki = lax.broadcasted_iota(i32, (128, 128), 0)
    qi = lax.broadcasted_iota(i32, (128, 128), 1)
    return ki <= qi


def _phi(t):
    return jnp.where(t > 0, t + 1.0, jnp.exp(jnp.minimum(t, 0.0))) + 1e-6


def _head_of(f):
    return lax.shift_right_logical(f * 2341, 16)


_B_ROWS = [(0, 144), (112, 288), (240, 400), (352, 448)]
_B_TILE = [(0, 128), (128, 256), (256, 384), (384, 448)]


def _kernel(xa_h, ckv_h, wq_h, wk_h, wv_h, wo_h, wqkv_h, wob_h, gw_h, out_h,
            xa, ckv, wq_raw, wk_raw, wv_raw, wo, wqkv, wsm, wob, gw,
            wqkvT, wsmT, wobT, gcol, kvacc, kvz, wqT, wk, wvT, qT, kk, vT, oT, acc, outs, sems, *, cfg):
    W, BK, DEPTH, CW = cfg["W"], cfg["BK"], cfg["DEPTH"], cfg["CW"]
    halves = lambda src, dst, s0: [
        pltpu.make_async_copy(src.bitcast(i32).at[:, pl.ds(t * 128, 128)], dst.at[t], sems.at[s0 + t])
        for t in range(2)]
    xcw = cfg["CW1"]
    cps = {
        "wqkv_kv": [pltpu.make_async_copy(wqkv_h.at[:, pl.ds(384, 3 * M - 384)], wqkv, sems.at[0])],
        "wqkv_q": [pltpu.make_async_copy(wqkv_h.at[:, pl.ds(0, 384)], wsm, sems.at[1])],
        "wob": [pltpu.make_async_copy(wob_h, wob, sems.at[2])],
        "gw": [pltpu.make_async_copy(gw_h, gw, sems.at[3])],
        "ckv": [pltpu.make_async_copy(ckv_h.bitcast(i32), ckv, sems.at[5])],
        "wq": halves(wq_h, wq_raw, 6),
        "wk": halves(wk_h, wk_raw, 8),
        "wv": halves(wv_h, wv_raw, 10),
        "wo": [pltpu.make_async_copy(wo_h.bitcast(i32), wo, sems.at[12])],
    }

    def xa_copy(i):
        col = pl.ds(pl.multiple_of(i * xcw, 128), xcw)
        return pltpu.make_async_copy(xa_h.bitcast(i32).at[:, col], xa.at[:, col], sems.at[21 + i])

    def start(*names):
        for name in names:
            for cp in cps[name]:
                cp.start()

    def wait(*names):
        for name in names:
            for cp in cps[name]:
                cp.wait()

    start("wqkv_kv")
    xa_copy(0).start()

    def unpack(w, sh):
        return pltpu.bitcast(lax.shift_left(w, jnp.broadcast_to(sh, w.shape)) & _HI_MASK, f32).astype(bf16)

    def wq_jobs(j):
        jobs = []
        for dt in range(2):
            for m0 in range(0, M, 128):
                mw = min(128, M - m0)

                def job(dt=dt, m0=m0, mw=mw):
                    w = wq_raw[dt, pl.ds(8 * m0 + j, mw, stride=8), :].T
                    wqT[dt * 64:(dt + 1) * 64, m0:m0 + mw] = _st(pltpu.bitcast(w << 16, f32).astype(bf16))
                    wqT[128 + dt * 64:128 + (dt + 1) * 64, m0:m0 + mw] = _st(
                        pltpu.bitcast(w & _HI_MASK, f32).astype(bf16))
                jobs.append(job)
        return jobs

    def wkv_jobs(h, part=None):
        j = h // 2
        sh = (1 - h % 2) * 16
        jobs = []
        for dt in range(2):
            for cb in (range(C // 128) if part is None else [4 * part + u for u in range(4)]):
                def job(dt=dt, cb=cb):
                    w = wk_raw[dt, pl.ds(1024 * cb + j, 128, stride=8), :]
                    rows = slice(cb * 64, (cb + 1) * 64) if part is None else pl.ds(pl.multiple_of(cb * 64, 64), 64)
                    wk[rows, dt * 128:(dt + 1) * 128] = _st(unpack(w, sh))
                jobs.append(job)

                def job2(dt=dt, cb=cb):
                    w = wv_raw[dt, pl.ds(1024 * cb + j, 128, stride=8), :]
                    wvT[cb, dt * 64:(dt + 1) * 64, :] = _st(unpack(w.T, sh))
                jobs.append(job2)
        return jobs

    wait("wqkv_kv")
    for i in range(1, S // xcw):
        xa_copy(i).start()
    for f0 in range(0, 3 * M - 384, 128):
        wdt = min(128, 3 * M - 384 - f0)
        wqkvT[f0 // 2:(f0 + wdt) // 2, :] = _st(wqkv[:, f0:f0 + wdt].astype(f32).T.astype(bf16))
    kvacc[...] = jnp.zeros(kvacc.shape, f32)
    start("wq", "wqkv_q", "wob", "gw")
    kv_off = [0, 160, 352, 528]
    NSUB = cfg["NSUB"]
    SW = CW // NSUB

    def b1_chunk(i, carry):
        xa_copy(i).wait()
        w_kv = _ld(wqkvT[32:32 + M, :])
        pend = []
        NS1 = xcw // SW
        for c in range(NS1 + 1):
            if c < NS1:
                x = _ld(xa[:, pl.ds(pl.multiple_of(i * xcw + c * SW, 128), SW)])
                kvt = _nn(w_kv, x)
                pend.append((_phi(kvt[:M]).astype(bf16), kvt[M:].astype(bf16)))
            if c >= 1:
                pk, v = pend.pop(0)
                ones = jnp.ones((16, SW), bf16)
                for j in range(4):
                    r0, r1 = _B_ROWS[j]
                    d0, d1 = _B_TILE[j]
                    part = _nt(jnp.concatenate([v[r0:r1], ones], axis=0), pk[d0:d1])
                    kvacc[kv_off[j]:kv_off[j] + r1 - r0 + 16, 0:d1 - d0] += part
        return carry

    lax.fori_loop(0, S // xcw, b1_chunk, 0)
    wait("wq")
    start("ckv", "wk", "wv", "wo")
    wait("wqkv_q", "wob", "gw")
    for job in wq_jobs(0):
        job()
    off = 0
    for j in range(4):
        r0, r1 = _B_ROWS[j]
        d0, d1 = _B_TILE[j]
        n = r1 - r0
        eh = _head_of(lax.broadcasted_iota(i32, (n, d1 - d0), 0) + r0)
        dh = _head_of(lax.broadcasted_iota(i32, (n, d1 - d0), 1) + d0)
        same = eh == dh
        kvj = kvacc[kv_off[j]:kv_off[j] + n + 16, 0:d1 - d0]
        kvm = jnp.where(same, kvj[:n], 0.0)
        hz = lax.broadcasted_iota(i32, (H, d1 - d0), 0) == _head_of(lax.broadcasted_iota(i32, (H, d1 - d0), 1) + d0)
        zm = jnp.where(hz, kvj[n:n + H], 0.0)
        kvz[off:off + (n + H) // 2, 0:d1 - d0] = _st(jnp.concatenate([kvm, zm], axis=0).astype(bf16))
        off += (n + H) // 2

    def q_pair(j, carry, late=False):
        w = _ld(wqT[:, :M])
        jobs = wq_jobs(jnp.minimum(j + 1, H // 2 - 1))
        kv_jobs = wkv_jobs(0, j - (H // 2 - 2)) if late else []
        jc = jnp.minimum(j, 2)
        rows, cols = pl.ds(pl.multiple_of(jc * 64, 64), 64), pl.ds(pl.multiple_of(jc * 128, 128), 128)
        wsmT[rows, :] = _st(wsm[:, cols].astype(f32).T.astype(bf16))
        wobT[rows, :] = _st(wob[:, cols].astype(f32).T.astype(bf16))
        wobT[192:224, :] = _st(wob[:, 384:M].astype(f32).T.astype(bf16))
        acc[:, pl.ds(pl.multiple_of(j * 256, 256), 256)] = jnp.zeros((M, 256), f32)
        gcol[...] = jnp.broadcast_to(gw[...].astype(f32).reshape(1, M), (128, M)).T
        for t in range(NT):
            q = _nn(w, _ld(xa[:, t * 128:(t + 1) * 128])) * (D ** -0.5 * LOG2E)
            q = _st(q.astype(bf16))
            qT[2 * j, t] = q[:128]
            qT[2 * j + 1, t] = q[128:]
            if t >= NT - len(jobs):
                jobs[t - (NT - len(jobs))]()
            if t < len(kv_jobs):
                kv_jobs[t]()
        return carry

    lax.fori_loop(0, H // 2 - 2, q_pair, 0)
    wait("ckv", "wk", "wv")
    lax.fori_loop(H // 2 - 2, H // 2, functools.partial(q_pair, late=True), 0)

    wait("wo")

    def head(h, carry):
        w_k = _ld(wk[...])
        for c in range(S // 256):
            kk[c * 128:(c + 1) * 128, :] = _st(_nn(_ld(ckv[c * 128:(c + 1) * 128, :]), w_k).astype(bf16))
        w_vT = jnp.concatenate([_ld(wvT[cb]) for cb in range(C // 128)], axis=1)
        for t in range(NT - 1, -1, -1):
            vT[t] = _st(_nt(w_vT, _ld(ckv[t * 64:(t + 1) * 64, :])).astype(bf16))

        tasks = []
        for qb in range(NT // W - 1, -1, -1):
            q0 = qb * W * 128
            for k0 in range(0, q0, BK):
                tasks.append(("full", qb, k0, min(BK, q0 - k0)))
            for t in range(W):
                tasks.append(("diag", qb, t))
        state = {}

        def tiles(get, t0, n):
            xs = [_ld(get(t)) for t in range(t0, t0 + n)]
            return jnp.concatenate(xs, axis=1) if n > 1 else xs[0]
        get_q = lambda t: qT[h, t]
        get_v = lambda t: vT[t]

        def do_qk(task):
            if task[0] == "full":
                _, qb, k0, nk = task
                s = _nn(_ld(kk[k0 // 2:(k0 + nk) // 2, :]), tiles(get_q, qb * W, W))
            else:
                _, qb, t = task
                q0, nk = qb * W * 128, 128 * (t + 1)
                s = _nn(_ld(kk[q0 // 2:(q0 + nk) // 2, :]), tiles(get_q, qb * W + t, 1))
                dg = jnp.where(_tri(), s[nk - 128:], NEG)
                s = jnp.concatenate([s[:nk - 128], dg], axis=0) if nk > 128 else dg
            return s, jnp.max(_red(jnp.maximum, s), axis=0, keepdims=True)

        def upd(st_, s, mx, v):
            if st_ is None:
                p = jnp.exp2(s - mx)
                return mx, _red(jnp.add, p), _nn(v, p.astype(bf16))
            m, l, a = st_
            m_new = jnp.maximum(m, mx)
            alpha = jnp.exp2(m - m_new)
            p = jnp.exp2(s - m_new)
            return m_new, alpha * l + _red(jnp.add, p), a * alpha + _nn(v, p.astype(bf16))

        def do_pv(task, s, mx):
            if task[0] == "full":
                _, qb, k0, nk = task
                state[qb] = upd(state.get(qb), s, mx, tiles(get_v, k0 // 128, nk // 128))
                return None
            _, qb, t = task
            full = state.get(qb)
            sl = slice(t * 128, (t + 1) * 128)
            st_ = None if full is None else tuple(x[:, sl] for x in full)
            _, l, a = upd(st_, s, mx, tiles(get_v, qb * W, t + 1))
            tt = qb * W + t
            scale = 1.0 / jnp.sum(l, axis=0, keepdims=True)
            oT[tt] = _st((a * scale).astype(bf16))
            return tt

        def out_proj(tt):
            w_o = _ld(wo[pl.ds(pl.multiple_of(h * (M // 2), 8), M // 2), :])
            acc[:, tt * 128:(tt + 1) * 128] += _nn(w_o, _ld(oT[tt]))

        jobs = wkv_jobs(jnp.minimum(h + 1, H - 1))
        n = len(tasks)
        per = -(-len(jobs) // n)
        pend, done = [], []
        for i in range(n + DEPTH):
            if i < n:
                pend.append((tasks[i],) + do_qk(tasks[i]))
            if i >= DEPTH:
                tt = do_pv(*pend.pop(0))
                if tt is not None:
                    done.append((i, tt))
            while done and (i - done[0][0] >= cfg["OLAG"]):
                out_proj(done.pop(0)[1])
            for job in jobs[i * per:(i + 1) * per]:
                job()
        for _, tt in done:
            out_proj(tt)
        return carry

    lax.fori_loop(0, H, head, 0)


    def merge(p):
        return jnp.concatenate([
            p[0][0:112], p[0][112:144] + p[1][0:32], p[1][32:128], p[1][128:176] + p[2][0:48],
            p[2][48:112], p[2][112:160] + p[3][0:48], p[3][48:96]], axis=0)

    def spread(r16):
        bc = [jnp.broadcast_to(r16[h:h + 1], (8, r16.shape[1])) for h in range(H)]
        low = lax.broadcasted_iota(i32, bc[0].shape, 0) < 4
        rows = []
        for r in range(0, M, 8):
            h0, h1 = r // DH, (r + 7) // DH
            rows.append(bc[h0] if h0 == h1 else jnp.where(low, bc[h0], bc[h1]))
        return jnp.concatenate(rows, axis=0)

    def out_copy(slot):
        col = pl.ds(pl.multiple_of(slot * SW, 128), SW)
        return pltpu.make_async_copy(outs.at[slot], out_h.bitcast(i32).at[:, col], sems.at[25 + slot])

    def b2_chunk(i, carry):
        w_q = jnp.concatenate([_ld(wsmT[...]), _ld(wqkvT[0:32, :])], axis=0)
        w_ob = _ld(wobT[...])
        lhs2, off = [], 0
        for j in range(4):
            n = _B_ROWS[j][1] - _B_ROWS[j][0]
            lhs2.append(_ld(kvz[off:off + (n + H) // 2, 0:_B_TILE[j][1] - _B_TILE[j][0]]))
            off += (n + H) // 2
        pa, pb = [], []
        for c in range(NSUB + 2):
            if c < NSUB:
                col = pl.ds(pl.multiple_of(i * CW + c * SW, 128), SW)
                x = _ld(xa[:, col])
                gs = []
                for t in range(SW // 128):
                    prod = x[:, t * 128:(t + 1) * 128].astype(f32) * gcol[...]
                    z = jnp.sum(jnp.sum(prod.reshape(M // 8, 8, 128), axis=0), axis=0, keepdims=True)
                    gs.append(jax.nn.sigmoid(z))
                g = jnp.concatenate(gs, axis=1) if len(gs) > 1 else gs[0]
                pa.append((_phi(_nn(w_q, x)).astype(bf16), g))
            if 1 <= c <= NSUB:
                pq, g = pa.pop(0)
                nums, dens = [], []
                for j in range(4):
                    n = _B_ROWS[j][1] - _B_ROWS[j][0]
                    d0, d1 = _B_TILE[j]
                    r = _nn(lhs2[j], pq[d0:d1])
                    nums.append(r[:n])
                    dens.append(r[n:])
                r16 = (1.0 - g) / ((dens[0] + dens[1]) + (dens[2] + dens[3]) + 1e-6)
                pb.append(((merge(nums) * spread(r16)).astype(bf16), g))
            if c >= 2:
                o, g = pb.pop(0)
                col = pl.ds(pl.multiple_of(i * CW + (c - 2) * SW, 128), SW)
                res = g * acc[:, col] + _nn(w_ob, o)
                slot = i * NSUB + c - 2
                outs[slot] = _st(res.astype(bf16))
                out_copy(slot).start()
        return carry

    lax.fori_loop(0, S // CW, b2_chunk, 0)

    for slot in range(S // SW):
        out_copy(slot).wait()


CFG = dict(W=2, BK=128, DEPTH=6, CW=512, NSUB=2, OLAG=8, CW1=512)


def build(cfg=CFG, name="fused"):
    def run(A_x, A_c_kv, A_w_q, A_w_uk, A_w_uv, A_w_o, B_x, B_wqkv, B_wo, gate_w):
        any_spec = pl.BlockSpec(memory_space=pl.ANY)
        VM = pltpu.VMEM
        outT = pl.pallas_call(
            functools.partial(_kernel, cfg=cfg),
            out_shape=jax.ShapeDtypeStruct((M, S), bf16),
            in_specs=[any_spec] * 9,
            out_specs=any_spec,
            scratch_shapes=[
                VM((M // 2, S), i32), VM((S // 2, C), i32),
                VM((2, M * 8, 128), i32), VM((2, C * 8, 128), i32), VM((2, C * 8, 128), i32),
                VM((H * M // 2, D), i32),
                VM((M, 3 * M - 384), bf16), VM((M, 384), bf16), VM((M, M), bf16), VM((M,), bf16),
                VM(((3 * M - 384) // 2, M), i32), VM((192, M), i32), VM((M // 2, M), i32), VM((M, 128), f32), VM((640, 128), f32), VM((576, 128), i32),
                VM((256, 512), i32), VM((C // 2, D), i32), VM((C // 128, 128, 128), i32),
                VM((H, NT, 128, 128), i32), VM((S // 2, D), i32), VM((NT, 128, 128), i32), VM((NT, 128, 128), i32),
                VM((M, S), f32), VM((S * cfg['NSUB'] // cfg['CW'], M // 2, cfg['CW'] // cfg['NSUB']), i32), pltpu.SemaphoreType.DMA((33,)),
            ],
            compiler_params=pltpu.CompilerParams(vmem_limit_bytes=110 * 1024 * 1024),
            name=name,
        )(
            A_x.reshape(S, M).T, A_c_kv.reshape(S, C), A_w_q.reshape(M * H, D),
            A_w_uk.reshape(C * H, D), A_w_uv.reshape(C * H, D),
            jnp.swapaxes(A_w_o, 1, 2).reshape(H * M, D), B_wqkv, B_wo, gate_w,
        )
        return outT.T.reshape(1, S, M)
    return run


@jax.jit
def pallas_gated_mix__compressed_kv_cla__linear_attn_block__prompt_kernel(
        A_x, A_c_kv, A_w_q, A_w_uk, A_w_uv, A_w_o, B_x, B_wqkv, B_wo, gate_w):
    return build()(A_x, A_c_kv, A_w_q, A_w_uk, A_w_uv, A_w_o, B_x, B_wqkv, B_wo, gate_w)
```
